```python
import jax
import jax.numpy as jnp

def _softmax(x, axis=-1):
    return jax.nn.softmax(x, axis=axis)
def _gelu(x):
    return jax.nn.gelu(x, approximate=True)
def _silu(x):
    return jax.nn.silu(x)
def _sigmoid(x):
    return jax.nn.sigmoid(x)
def _layernorm(x, axis=-1, eps=1e-5):
    m = jnp.mean(x, axis=axis, keepdims=True)
    v = jnp.var(x, axis=axis, keepdims=True)
    return (x - m) / jnp.sqrt(v + eps)
def _scatter_add(tgt, idx, src, axis=0):
    return tgt.at[idx].add(src)
def _segment_sum(src, seg, n):
    return jax.ops.segment_sum(src, seg, n)
class _Rng:
    def __init__(self, key):
        self._k = key
    def _next(self):
        self._k, sub = jax.random.split(self._k)
        return sub
    def normal(self, shape):
        return jax.random.normal(self._next(), shape, dtype=jnp.bfloat16)
    def randint(self, lo, hi, shape):
        return jax.random.randint(self._next(), shape, lo, hi, dtype=jnp.int32)
    def uniform(self, shape, lo=0.0, hi=1.0):
        return jax.random.uniform(self._next(), shape, jnp.bfloat16, lo, hi)
    def permutation(self, n):
        return jax.random.permutation(self._next(), n)


kernel_name = 'sequential_preLN__linear_attn_block__moe_arch_mod__prompt'

def setup_inputs():
    _rng = _Rng(jax.random.key(int.from_bytes(__import__("os").urandom(4), "little")))
    _w = (lambda a: (lambda t: t.astype(jnp.bfloat16) if jnp.issubdtype(t.dtype, jnp.floating) else t)(jnp.asarray(a)))
    def _A_setup():
        B, S, D = 1, 2048, 1024
        return {
            "x": _w((lambda *s: _rng.normal(s) * 0.05)(B, S, D)),
            "wqkv": _w((lambda *s: _rng.normal(s) * 0.05)(D, 3 * D)),
            "wo": _w((lambda *s: _rng.normal(s) * 0.05)(D, D)),
        }
    _A_in = _A_setup()

    def _B_setup():
        B, S, D, F, C = 1, 2048, 1024, 3584, 2
        return {
            "x": _w((lambda *s: _rng.normal(s) * 0.05)(B, S, D)),
            "w_r": _w((lambda *s: _rng.normal(s) * 0.05)(D)),
            "w_gate": _w((lambda *s: _rng.normal(s) * 0.05)(D, F)),
            "w_up": _w((lambda *s: _rng.normal(s) * 0.05)(D, F)),
            "w_down": _w((lambda *s: _rng.normal(s) * 0.05)(F, D)),
        }
    _B_in = _B_setup()

    return {
        "A_x": _A_in["x"],
        "A_wqkv": _A_in["wqkv"],
        "A_wo": _A_in["wo"],
        "B_x": _B_in["x"],
        "B_w_r": _B_in["w_r"],
        "B_w_gate": _B_in["w_gate"],
        "B_w_up": _B_in["w_up"],
        "B_w_down": _B_in["w_down"],
    }

def reference(A_x, A_wqkv, A_wo, B_x, B_w_r, B_w_gate, B_w_up, B_w_down):
    def _A_ref(x, wqkv, wo):
        B, S, D = x.shape
        H = 32; Dh = D // H
        qkv = (lambda x, *d: x.transpose(*d))((x @ wqkv).reshape(B, S, 3, H, Dh), 2, 0, 3, 1, 4)
        q, k, v = qkv[0], qkv[1], qkv[2]
        phi = lambda t: jnp.where(t > 0, t + 1, jnp.exp(t)) + 1e-6
        pq, pk = phi(q), phi(k)
        kv = jnp.einsum("bhsd,bhse->bhde", pk, v)
        z = jnp.einsum("bhsd->bhd", pk)
        num = jnp.einsum("bhqd,bhde->bhqe", pq, kv)
        den = jnp.einsum("bhqd,bhd->bhq", pq, z)[..., None] + 1e-6
        o = num / den
        return (lambda x, *d: x.transpose(*d))(o, 0, 2, 1, 3).reshape(B, S, D) @ wo

    def _B_ref(x, w_r, w_gate, w_up, w_down):
        B, S, D = x.shape
        C = 2
        r = x @ w_r
        idx = jnp.argsort(-r, axis=-1)[:, :C]
        idx_e = jnp.repeat(idx.reshape(B, C, 1), D, axis=2)
        x_sel = jnp.take_along_axis(x, idx_e, axis=1)
        g = _silu(x_sel @ w_gate)
        u = x_sel @ w_up
        y = (g * u) @ w_down
        r_sel = _sigmoid(jnp.take_along_axis(r, idx, axis=1))
        y = y * r_sel.reshape(B, C, 1)
        b_off = (jnp.arange(B) * S).reshape(B, 1)
        flat_idx = (idx + b_off).reshape(B * C)
        zero = (x * 0.0).reshape(B * S, D)
        upd = _scatter_add(zero, flat_idx, y.reshape(B * C, D), axis=0)
        return x + upd.reshape(B, S, D)

    x = A_x
    h = x + _A_ref(_layernorm(x, axis=-1), A_wqkv, A_wo)
    h2 = h + _B_ref(_layernorm(h, axis=-1), B_w_r, B_w_gate, B_w_up, B_w_down)
    return h2
```

```python
import jax
import jax.numpy as jnp
from jax import lax
import jax.experimental.pallas as pl
import jax.experimental.pallas.tpu as pltpu

S, D, F, H = 2048, 1024, 3584, 32
DH = D // H
TM = 512
NT = S // TM
MODE = 'T'
f32, bf16 = jnp.float32, jnp.bfloat16


def _ln(x):
    m = jnp.mean(x, axis=-1, keepdims=True)
    xc = x - m
    v = jnp.mean(xc * xc, axis=-1, keepdims=True)
    return xc * lax.rsqrt(v + 1e-5)


def _phi(t):
    return jnp.where(t > 0, t + 1.0, jnp.exp(t)) + 1e-6


def _kernel(x_hbm, wqkv_hbm, wo_hbm, wr_ref, wg_hbm, wu_hbm, wd_hbm, out_hbm,
            x_v, xn_v, wqkv_v, wo_v, wg_v, wu_v, wd_v, out_v, acc_v, z_v, m_v, zm_v, r_v,
            sem_x, sem_w, sem_o):
    def xcp(i):
        return pltpu.make_async_copy(x_hbm.at[pl.ds(i * TM, TM)], x_v.at[pl.ds(i * TM, TM)], sem_x.at[i])
    def wcp(j):
        return pltpu.make_async_copy(wqkv_hbm.at[:, pl.ds(j * D, D)], wqkv_v.at[:, pl.ds(j * D, D)], sem_w.at[j])
    cp_wo = pltpu.make_async_copy(wo_hbm, wo_v, sem_w.at[3])
    cp_wg = pltpu.make_async_copy(wg_hbm, wg_v, sem_w.at[4])
    cp_wu = pltpu.make_async_copy(wu_hbm, wu_v, sem_w.at[5])
    cp_wd = pltpu.make_async_copy(wd_hbm, wd_v, sem_w.at[6])
    def ocp(i):
        return pltpu.make_async_copy(out_v.at[pl.ds(i * TM, TM)], out_hbm.at[pl.ds(i * TM, TM)], sem_o.at[i])

    xcp(0).start()
    wcp(1).start()
    for i in range(1, NT):
        xcp(i).start()
    wcp(2).start()
    wcp(0).start()
    cp_wo.start()
    cp_wg.start()
    cp_wu.start()
    cp_wd.start()

    ri = lax.broadcasted_iota(jnp.int32, (128, 128), 0) // DH
    ci = lax.broadcasted_iota(jnp.int32, (128, 128), 1) // DH
    hmask = ri == ci

    acc_v[...] = jnp.zeros_like(acc_v)
    z_v[...] = jnp.zeros_like(z_v)

    def p1(i, c):
        xcp(i).wait()
        rows = pl.ds(pl.multiple_of(i * TM, TM), TM)
        xn = _ln(x_v[rows, :].astype(f32)).astype(bf16)
        xn_v[rows, :] = xn
        @pl.when(i == 0)
        def _():
            wcp(1).wait()
        k = jnp.dot(xn, wqkv_v[:, D:2 * D], preferred_element_type=f32)
        pk = _phi(k)
        z_v[...] += jnp.sum(pk.reshape(TM // 8, 8, D), axis=0)
        pkb = pk.astype(bf16)
        if MODE == 'T':
            acc_v[...] += lax.dot_general(pkb, xn, (((0,), (0,)), ((), ())), preferred_element_type=f32)
        else:
            @pl.when(i == 0)
            def _():
                wcp(2).wait()
            v = jnp.dot(xn, wqkv_v[:, 2 * D:], preferred_element_type=f32).astype(bf16)
            for b in range(8):
                sl = slice(b * 128, (b + 1) * 128)
                acc_v[:, sl] += lax.dot_general(pkb[:, sl], v[:, sl], (((0,), (0,)), ((), ())), preferred_element_type=f32)
        return c
    lax.fori_loop(0, NT, p1, 0)

    if MODE == 'T':
        wcp(2).wait()
    cp_wo.wait()
    z = jnp.sum(z_v[...], axis=0, keepdims=True)
    for b in range(8):
        sl = slice(b * 128, (b + 1) * 128)
        if MODE == 'T':
            kvb = jnp.dot(acc_v[sl, :].astype(bf16), wqkv_v[:, 2 * D + b * 128:2 * D + (b + 1) * 128], preferred_element_type=f32)
        else:
            kvb = acc_v[:, sl]
        kvb = jnp.where(hmask, kvb, 0.0).astype(bf16)
        m_v[sl, :] = jnp.dot(kvb, wo_v[sl, :], preferred_element_type=f32).astype(bf16)
        zrow = jnp.broadcast_to(z[:, sl], (128, 128))
        zm_v[:, sl] = jnp.where(hmask, zrow.T, 0.0).astype(bf16)

    wcp(0).wait()
    wr = wr_ref[...].astype(f32)
    lane = lax.broadcasted_iota(jnp.int32, (8, 128), 1)

    def p2(i, c):
        rows = pl.ds(pl.multiple_of(i * TM, TM), TM)
        xn = xn_v[rows, :]
        q = jnp.dot(xn, wqkv_v[:, :D], preferred_element_type=f32)
        pq = _phi(q)
        pqb = pq.astype(bf16)
        dens = []
        for b in range(8):
            sl = slice(b * 128, (b + 1) * 128)
            dens.append(jnp.dot(pqb[:, sl], zm_v[:, sl], preferred_element_type=f32))
        den = jnp.concatenate(dens, axis=1) + 1e-6
        a = (pqb.astype(f32) / den).astype(bf16)
        h = x_v[rows, :].astype(f32) + jnp.dot(a, m_v[...], preferred_element_type=f32)
        hn = _ln(h)
        hnb = hn.astype(bf16)
        xn_v[rows, :] = hnb
        out_v[rows, :] = (h + hn).astype(bf16)
        ocp(i).start()
        hf = hnb.astype(f32)
        racc = hf[:, 0:128] * wr[0:1, :]
        for b in range(1, 8):
            racc = racc + hf[:, b * 128:(b + 1) * 128] * wr[b:b + 1, :]
        r = jnp.sum(racc, axis=-1, keepdims=True)
        nv = TM // 8
        blk = (i * nv) // 128
        off = (i * nv) % 128
        cur = r_v[blk]
        for j in range(nv):
            cur = jnp.where(lane == off + j, jnp.broadcast_to(r[j * 8:(j + 1) * 8, :], (8, 128)), cur)
        r_v[blk] = cur
        return c
    r_v[...] = jnp.zeros_like(r_v)
    lax.fori_loop(0, NT, p2, 0)

    rv = jnp.concatenate([r_v[0], r_v[1]], axis=1)
    sub = lax.broadcasted_iota(jnp.int32, (8, 256), 0)
    ln2 = lax.broadcasted_iota(jnp.int32, (8, 256), 1)
    tok = ln2 * 8 + sub
    m0 = jnp.max(rv)
    i0 = jnp.min(jnp.where(rv == m0, tok, S))
    rv1 = jnp.where(tok == i0, -jnp.inf, rv)
    m1 = jnp.max(rv1)
    i1 = jnp.min(jnp.where(rv1 == m1, tok, S))
    b0 = pl.multiple_of((i0 // 16) * 16, 16)
    b1 = pl.multiple_of((i1 // 16) * 16, 16)
    r16 = lax.broadcasted_iota(jnp.int32, (16, D), 0)
    blk0 = xn_v[pl.ds(b0, 16), :].astype(f32)
    blk1 = xn_v[pl.ds(b1, 16), :].astype(f32)
    row0 = jnp.sum(jnp.where(r16 == i0 - b0, blk0, 0.0), axis=0, keepdims=True)
    row1 = jnp.sum(jnp.where(r16 == i1 - b1, blk1, 0.0), axis=0, keepdims=True)
    r8 = lax.broadcasted_iota(jnp.int32, (8, D), 0)
    xs = jnp.where(r8 == 0, row0, jnp.where(r8 == 1, row1, 0.0)).astype(bf16)
    cp_wg.wait()
    cp_wu.wait()
    g = jnp.dot(xs, wg_v[...], preferred_element_type=f32)
    u = jnp.dot(xs, wu_v[...], preferred_element_type=f32)
    act = (g * jax.nn.sigmoid(g) * u).astype(bf16)
    cp_wd.wait()
    y = jnp.dot(act, wd_v[...], preferred_element_type=f32)
    y0 = y[0:1, :] * jax.nn.sigmoid(jnp.full((1, D), m0, f32))
    y1 = y[1:2, :] * jax.nn.sigmoid(jnp.full((1, D), m1, f32))
    for i in range(NT):
        ocp(i).wait()
    o0 = out_v[pl.ds(b0, 16), :].astype(f32)
    out_v[pl.ds(b0, 16), :] = jnp.where(r16 == i0 - b0, o0 + y0, o0).astype(bf16)
    o1 = out_v[pl.ds(b1, 16), :].astype(f32)
    out_v[pl.ds(b1, 16), :] = jnp.where(r16 == i1 - b1, o1 + y1, o1).astype(bf16)
    c0 = pltpu.make_async_copy(out_v.at[pl.ds(b0, 16)], out_hbm.at[pl.ds(b0, 16)], sem_w.at[7])
    c1 = pltpu.make_async_copy(out_v.at[pl.ds(b1, 16)], out_hbm.at[pl.ds(b1, 16)], sem_w.at[8])
    c0.start()
    @pl.when(b1 != b0)
    def _():
        c1.start()
        c1.wait()
    c0.wait()


@jax.jit
def pallas_sequential_preLN__linear_attn_block__moe_arch_mod__prompt_kernel(
        A_x, A_wqkv, A_wo, B_x, B_w_r, B_w_gate, B_w_up, B_w_down):
    del B_x
    x = A_x.reshape(S, D)
    wr = B_w_r.reshape(8, 128)
    anyspec = pl.BlockSpec(memory_space=pl.ANY)
    accshape = (D, D) if MODE == 'T' else (128, D)
    out = pl.pallas_call(
        _kernel,
        out_shape=jax.ShapeDtypeStruct((S, D), bf16),
        in_specs=[anyspec, anyspec, anyspec, pl.BlockSpec(memory_space=pltpu.VMEM), anyspec, anyspec, anyspec],
        out_specs=anyspec,
        scratch_shapes=[
            pltpu.VMEM((S, D), bf16), pltpu.VMEM((S, D), bf16), pltpu.VMEM((D, 3 * D), bf16),
            pltpu.VMEM((D, D), bf16), pltpu.VMEM((D, F), bf16), pltpu.VMEM((D, F), bf16),
            pltpu.VMEM((F, D), bf16), pltpu.VMEM((S, D), bf16),
            pltpu.VMEM(accshape, f32), pltpu.VMEM((8, D), f32), pltpu.VMEM((D, D), bf16),
            pltpu.VMEM((128, D), bf16), pltpu.VMEM((2, 8, 128), f32),
            pltpu.SemaphoreType.DMA((NT,)), pltpu.SemaphoreType.DMA((9,)), pltpu.SemaphoreType.DMA((NT,)),
        ],
        compiler_params=pltpu.CompilerParams(vmem_limit_bytes=100 * 1024 * 1024),
    )(x, A_wqkv, A_wo, wr, B_w_gate, B_w_up, B_w_down)
    return out.reshape(1, S, D)
```

```python
import jax
import jax.numpy as jnp
from jax import lax
import jax.experimental.pallas as pl
import jax.experimental.pallas.tpu as pltpu

S, D, F, H = 2048, 1024, 3584, 32
DH = D // H
TM = 256
TH = TM // 2
DHALF = D // 2
NT = S // TM
JB = 128
RB = 128
f32, bf16 = jnp.float32, jnp.bfloat16
NN = (((1,), (0,)), ((), ()))
NT_ = (((1,), (1,)), ((), ()))


def _dot(a, b, dims=NN):
    return lax.dot_general(a, b, dims, preferred_element_type=f32)


def _ln(x):
    m = jnp.mean(x, axis=-1, keepdims=True)
    xc = x - m
    v = jnp.mean(xc * xc, axis=-1, keepdims=True)
    return xc * lax.rsqrt(v + 1e-5)


def _phi(t):
    return jnp.where(t > 0, t + 1.0, jnp.exp(t)) + 1e-6


def _aforms(a11, a12, a21, a22):
    return [a11 + a22, a21 + a22, a11, a22, a11 + a12, a21 - a11, a12 - a22]


def _bforms(b11, b12, b21, b22):
    return [b11 + b22, b11, b12 - b22, b21 - b11, b22, b11 + b12, b21 + b22]


A2B = [0, 2, 6, 5, 3, 4, 1]


def _combine(p):
    c11 = p[0] + p[3] - p[4] + p[6]
    c12 = p[2] + p[4]
    c21 = p[1] + p[3]
    c22 = p[0] - p[1] + p[2] + p[5]
    return c11, c12, c21, c22


def _stream(prod):
    p = prod(0); c11 = p; c22 = p
    p = prod(6); c11 = c11 + p
    p = prod(5); c22 = c22 + p
    p = prod(3); c11 = c11 + p; c21 = p
    p = prod(1); c21 = c21 + p; c22 = c22 - p
    p = prod(4); c11 = c11 - p; c12 = p
    p = prod(2); c12 = c12 + p; c22 = c22 + p
    return c11, c12, c21, c22


def _kernel(x_hbm, wqkv_hbm, wo_hbm, wr_ref, wg_hbm, wu_hbm, wd_hbm, out_hbm,
            x_v, xfE, xfO, wqkv_v, wo_v, wg_v, wu_v, wd_v, out_v, wkT_v, wqT_v, acc_v, z_v, mf_v, afE, afO, hn_v, hE, hO, r_v,
            sem_x, sem_w, sem_o, sem_f):
    def xcp(i):
        return pltpu.make_async_copy(x_hbm.at[pl.ds(i * TM, TM)], x_v.at[pl.ds(i * TM, TM)], sem_x.at[i])
    def wcp(j):
        return pltpu.make_async_copy(wqkv_hbm.at[:, pl.ds(j * D, D)], wqkv_v.at[:, pl.ds(j * D, D)], sem_w.at[j])
    cp_wo = pltpu.make_async_copy(wo_hbm, wo_v, sem_w.at[3])
    fcps = [pltpu.make_async_copy(wg_hbm, wg_v, sem_f.at[0]), pltpu.make_async_copy(wu_hbm, wu_v, sem_f.at[1]),
            ] + [pltpu.make_async_copy(wd_hbm.at[:, pl.ds(j * 128, 128)], wd_v.at[j], sem_f.at[2 + j]) for j in range(D // 128)]
    def ocp(i):
        return pltpu.make_async_copy(out_v.at[pl.ds(i * TM, TM)], out_hbm.at[pl.ds(i * TM, TM)], sem_o.at[i])

    xcp(0).start()
    wcp(1).start()

    NJ = DHALF // JB

    def ln_part(i, dst, part, nparts):
        base = i * TM
        ng = TH // 16
        for g in range(part * ng // nparts, (part + 1) * ng // nparts):
            xa = _ln(x_v[pl.ds(pl.multiple_of(base + g * 16, 16), 16), :].astype(f32))
            xb = _ln(x_v[pl.ds(pl.multiple_of(base + TH + g * 16, 16), 16), :].astype(f32))
            fs = _aforms(xa[:, :DHALF], xa[:, DHALF:], xb[:, :DHALF], xb[:, DHALF:])
            for n, fm in enumerate(fs):
                dst[n, g * 16:(g + 1) * 16, :] = fm.astype(bf16)

    def w_forms(dst, col0, b):
        for a in range(DHALF // 128):
            def blk(r, c):
                return wqkv_v[r * DHALF + a * 128:r * DHALF + (a + 1) * 128,
                              col0 + c * DHALF + b * 128:col0 + c * DHALF + (b + 1) * 128].astype(f32)
            fs = _bforms(blk(0, 0), blk(0, 1), blk(1, 0), blk(1, 1))
            for n, fm in enumerate(fs):
                dst[n, b * 128:(b + 1) * 128, a * 128:(a + 1) * 128] = fm.astype(bf16).T

    def proj(wT, xf, j):
        rows = slice(j * JB, (j + 1) * JB)
        c11, c12, c21, c22 = _stream(lambda n: _dot(wT[n, rows, :], xf[n], NT_))
        return c11, c21, c12, c22

    def k_tile(xf, extra, first=False):
        for j in range(NJ):
            rows = slice(j * JB, (j + 1) * JB)
            k11, k12, k21, k22 = [_phi(t) for t in proj(wkT_v, xf, j)]
            if first:
                z_v[0, rows, :] = k11 + k12
                z_v[1, rows, :] = k21 + k22
            else:
                z_v[0, rows, :] += k11 + k12
                z_v[1, rows, :] += k21 + k22
            fs = _aforms(k11, k12, k21, k22)
            for n, fm in enumerate(fs):
                t = _dot(fm.astype(bf16), xf[A2B[n]])
                if first:
                    acc_v[n, rows, :] = t
                else:
                    acc_v[n, rows, :] += t
            extra(j)

    xcp(0).wait()
    ln_part(0, xfE.at[0], 0, 1)
    wcp(1).wait()
    for i in range(1, NT):
        xcp(i).start()
    w_forms(wkT_v, D, 0)
    def ex0(j):
        b = (j + 1) * JB // 128
        if (j + 1) * JB % 128 == 0 and b < DHALF // 128:
            w_forms(wkT_v, D, b)
        if j == 0:
            xcp(1).wait()
        if j < NJ - 1:
            ln_part(1, xfO.at[0], j, NJ - 1)
    with jax.named_scope('k0'):
        k_tile(xfE.at[0], ex0, first=True)

    wcp(0).start()
    wcp(2).start()
    cp_wo.start()
    for c in fcps[:2]:
        c.start()

    def p1(m, c):
        xcp(2 * m + 2).wait()
        k_tile(xfO.at[m], lambda j: ln_part(2 * m + 2, xfE.at[m + 1], j, NJ))
        xcp(2 * m + 3).wait()
        k_tile(xfE.at[m + 1], lambda j: ln_part(2 * m + 3, xfO.at[m + 1], j, NJ))
        return c
    with jax.named_scope('p1'):
        lax.fori_loop(0, NT // 2 - 1, p1, 0)

    with jax.named_scope('mid'):
        wcp(0).wait()
        def exl(j):
            if (j + 1) * JB % 128 == 0:
                w_forms(wqT_v, 0, j * JB // 128)
        k_tile(xfO.at[NT // 2 - 1], exl)
        wcp(2).wait()
        cp_wo.wait()
        for c in fcps[2:]:
            c.start()
        ri = lax.broadcasted_iota(jnp.int32, (128, 128), 0) // DH
        ci = lax.broadcasted_iota(jnp.int32, (128, 128), 1) // DH
        hmask = ri == ci
        for hf in range(2):
            z_v[hf] = jnp.broadcast_to(jnp.sum(z_v[hf], axis=1, keepdims=True), (DHALF, 128))
        for b in range(DHALF // 128):
            sl = slice(b * 128, (b + 1) * 128)
            t11, t12, t21, t22 = _combine([acc_v[n, sl, :] for n in range(7)])
            ms = []
            for hf, (ta, tb) in enumerate(((t11, t12), (t21, t22))):
                c0 = hf * DHALF + b * 128
                tt = jnp.concatenate([ta, tb], axis=1).astype(bf16)
                kvb = _dot(tt, wqkv_v[:, 2 * D + c0:2 * D + c0 + 128])
                kvb = jnp.where(hmask, kvb, 0.0).astype(bf16)
                ms.append(_dot(kvb, wo_v[c0:c0 + 128, :]))
            fs = _bforms(ms[0][:, :DHALF], ms[0][:, DHALF:], ms[1][:, :DHALF], ms[1][:, DHALF:])
            for n, fm in enumerate(fs):
                mf_v[n, sl, :] = fm.astype(bf16)

    wr = wr_ref[...].astype(f32)
    lane = lax.broadcasted_iota(jnp.int32, (8, 128), 1)
    NP = 4

    def stage_a(xf, af, part):
        fparts = []
        for j in range(part * 128 // JB, (part + 1) * 128 // JB):
            rows = slice(j * JB, (j + 1) * JB)
            qs = proj(wqT_v, xf, j)
            a = []
            for n, t in enumerate(qs):
                pq = _phi(t)
                w = (pq * z_v[n // 2, rows, :]).reshape(JB // DH, DH, 128)
                den = jnp.sum(w, axis=1, keepdims=True) + 1e-6
                inv = pl.reciprocal(den, approx=True)
                inv = inv + inv * (1.0 - den * inv)
                a.append((pq.reshape(JB // DH, DH, 128) * inv).reshape(JB, 128))
            fparts.append([fm.astype(bf16) for fm in _aforms(a[0], a[2], a[1], a[3])])
        for n in range(7):
            af[n, :, part * 128:(part + 1) * 128] = jnp.concatenate([fp[n] for fp in fparts], axis=0).T

    def stage_b(af, h, part):
        cols = slice(part * 128, (part + 1) * 128)
        for r in range(TH // RB):
            rows = slice(r * RB, (r + 1) * RB)
            c11, c12, c21, c22 = _stream(lambda n: _dot(af[n, rows, :], mf_v[n, :, cols]))
            h[r * RB:(r + 1) * RB, part * 128:(part + 1) * 128] = c11
            h[r * RB:(r + 1) * RB, DHALF + part * 128:DHALF + (part + 1) * 128] = c12
            h[TH + r * RB:TH + (r + 1) * RB, part * 128:(part + 1) * 128] = c21
            h[TH + r * RB:TH + (r + 1) * RB, DHALF + part * 128:DHALF + (part + 1) * 128] = c22

    def stage_c(i, hbuf, part):
        base = i * TM
        nv = TM // 8
        blk = (i * nv) // 128
        off = (i * nv) % 128
        cur = r_v[blk]
        ng = TM // 16
        for g in range(part * ng // NP, (part + 1) * ng // NP):
            rows = pl.ds(pl.multiple_of(base + g * 16, 16), 16)
            h = x_v[rows, :].astype(f32) + hbuf[g * 16:(g + 1) * 16, :]
            hn = _ln(h)
            hn_v[rows, :] = hn.astype(bf16)
            out_v[rows, :] = (h + hn).astype(bf16)
            racc = hn[:, 0:128] * wr[0:1, :]
            for b in range(1, 8):
                racc = racc + hn[:, b * 128:(b + 1) * 128] * wr[b:b + 1, :]
            r = jnp.sum(racc, axis=-1, keepdims=True)
            for u in range(2):
                cur = jnp.where(lane == off + 2 * g + u, jnp.broadcast_to(r[u * 8:(u + 1) * 8, :], (8, 128)), cur)
        r_v[blk] = cur

    def step(a=None, b=None, c=None):
        for part in range(NP):
            if a is not None:
                stage_a(*a, part)
            if b is not None:
                stage_b(*b, part)
            if c is not None:
                stage_c(*c, part)
        if c is not None:
            ocp(c[0]).start()

    r_v[...] = jnp.zeros_like(r_v)
    with jax.named_scope('a01'):
        step(a=(xfE.at[0], afE))
        step(a=(xfO.at[0], afO), b=(afE, hE))

    def p2(m, c):
        step(a=(xfE.at[m + 1], afE), b=(afO, hO), c=(2 * m, hE))
        step(a=(xfO.at[m + 1], afO), b=(afE, hE), c=(2 * m + 1, hO))
        return c
    with jax.named_scope('p2'):
        lax.fori_loop(0, NT // 2 - 1, p2, 0)
    with jax.named_scope('p2e'):
        step(b=(afO, hO), c=(NT - 2, hE))
        step(c=(NT - 1, hO))

    with jax.named_scope('ffn'):
        rv = jnp.concatenate([r_v[0], r_v[1]], axis=1)
        sub = lax.broadcasted_iota(jnp.int32, (8, 256), 0)
        ln2 = lax.broadcasted_iota(jnp.int32, (8, 256), 1)
        tok = ln2 * 8 + sub
        m0 = jnp.max(rv)
        i0 = jnp.min(jnp.where(rv == m0, tok, S - 1))
        rv1 = jnp.where(tok == i0, -jnp.inf, rv)
        m1 = jnp.max(rv1)
        i1 = jnp.min(jnp.where(rv1 == m1, tok, S - 1))
        b0 = pl.multiple_of((i0 // 16) * 16, 16)
        b1 = pl.multiple_of((i1 // 16) * 16, 16)
        r16 = lax.broadcasted_iota(jnp.int32, (16, D), 0)
        blk0 = hn_v[pl.ds(b0, 16), :].astype(f32)
        blk1 = hn_v[pl.ds(b1, 16), :].astype(f32)
        row0 = jnp.sum(jnp.where(r16 == i0 - b0, blk0, 0.0), axis=0, keepdims=True)
        row1 = jnp.sum(jnp.where(r16 == i1 - b1, blk1, 0.0), axis=0, keepdims=True)
        r8 = lax.broadcasted_iota(jnp.int32, (8, D), 0)
        xs = jnp.where(r8 == 0, row0, jnp.where(r8 == 1, row1, 0.0)).astype(bf16)
        for c in fcps:
            c.wait()
        acts = []
        for j in range(F // 128):
            g = _dot(xs, wg_v[:, j * 128:(j + 1) * 128])
            u = _dot(xs, wu_v[:, j * 128:(j + 1) * 128])
            acts.append((g * jax.nn.sigmoid(g) * u).astype(bf16))
        act = jnp.concatenate(acts, axis=1)
        y = jnp.concatenate([_dot(act, wd_v[j]) for j in range(D // 128)], axis=1)
        y0 = y[0:1, :] * jax.nn.sigmoid(jnp.full((1, D), m0, f32))
        y1 = y[1:2, :] * jax.nn.sigmoid(jnp.full((1, D), m1, f32))
    with jax.named_scope('fin'):
        for i in range(NT):
            ocp(i).wait()
        o0 = out_v[pl.ds(b0, 16), :].astype(f32)
        out_v[pl.ds(b0, 16), :] = jnp.where(r16 == i0 - b0, o0 + y0, o0).astype(bf16)
        o1 = out_v[pl.ds(b1, 16), :].astype(f32)
        out_v[pl.ds(b1, 16), :] = jnp.where(r16 == i1 - b1, o1 + y1, o1).astype(bf16)
        c0 = pltpu.make_async_copy(out_v.at[pl.ds(b0, 16)], out_hbm.at[pl.ds(b0, 16)], sem_w.at[4])
        c1 = pltpu.make_async_copy(out_v.at[pl.ds(b1, 16)], out_hbm.at[pl.ds(b1, 16)], sem_w.at[5])
        c0.start()
        @pl.when(b1 != b0)
        def _():
            c1.start()
            c1.wait()
        c0.wait()


@jax.jit
def pallas_sequential_preLN__linear_attn_block__moe_arch_mod__prompt_kernel(
        A_x, A_wqkv, A_wo, B_x, B_w_r, B_w_gate, B_w_up, B_w_down):
    del B_x
    x = A_x.reshape(S, D)
    wr = B_w_r.reshape(8, 128)
    anyspec = pl.BlockSpec(memory_space=pl.ANY)
    V = pltpu.VMEM
    out = pl.pallas_call(
        _kernel,
        out_shape=jax.ShapeDtypeStruct((S, D), bf16),
        in_specs=[anyspec, anyspec, anyspec, pl.BlockSpec(memory_space=pltpu.VMEM), anyspec, anyspec, anyspec],
        out_specs=anyspec,
        scratch_shapes=[
            V((S, D), bf16), V((NT // 2, 7, TH, DHALF), bf16), V((NT // 2, 7, TH, DHALF), bf16), V((D, 3 * D), bf16),
            V((D, D), bf16), V((D, F), bf16), V((D, F), bf16),
            V((D // 128, F, 128), bf16), V((S, D), bf16),
            V((7, DHALF, DHALF), bf16), V((7, DHALF, DHALF), bf16),
            V((7, DHALF, DHALF), f32), V((2, DHALF, 128), f32), V((7, DHALF, DHALF), bf16),
            V((7, TH, DHALF), bf16), V((7, TH, DHALF), bf16), V((S, D), bf16), V((TM, D), f32), V((TM, D), f32), V((2, 8, 128), f32),
            pltpu.SemaphoreType.DMA((NT,)), pltpu.SemaphoreType.DMA((6,)), pltpu.SemaphoreType.DMA((NT,)),
            pltpu.SemaphoreType.DMA((10,)),
        ],
        compiler_params=pltpu.CompilerParams(vmem_limit_bytes=110 * 1024 * 1024, flags={"XLA_TPU_EVENLY_DISTRIBUTE_CRITICAL_NODES": True}),
    )(x, A_wqkv, A_wo, wr, B_w_gate, B_w_up, B_w_down)
    return out.reshape(1, S, D)
```
